```python
import os as _os
_os.environ.setdefault("JAX_PLATFORMS", "cpu")
import jax
import jax.numpy as jnp

def _softmax(x, axis=-1):
    return jax.nn.softmax(x, axis=axis)
def _gelu(x):
    return jax.nn.gelu(x, approximate=True)
def _silu(x):
    return jax.nn.silu(x)
def _sigmoid(x):
    return jax.nn.sigmoid(x)
def _layernorm(x, axis=-1, eps=1e-5):
    m = jnp.mean(x, axis=axis, keepdims=True)
    v = jnp.var(x, axis=axis, keepdims=True)
    return (x - m) / jnp.sqrt(v + eps)
def _scatter_add(tgt, idx, src, axis=0):
    return tgt.at[idx].add(src)
def _segment_sum(src, seg, n):
    return jax.ops.segment_sum(src, seg, n)
class _Rng:
    def __init__(self, key):
        self._k = key
    def _next(self):
        self._k, sub = jax.random.split(self._k)
        return sub
    def normal(self, shape):
        return jax.random.normal(self._next(), shape, dtype=jnp.bfloat16)
    def randint(self, lo, hi, shape):
        return jax.random.randint(self._next(), shape, lo, hi, dtype=jnp.int32)
    def uniform(self, shape, lo=0.0, hi=1.0):
        return jax.random.uniform(self._next(), shape, jnp.bfloat16, lo, hi)
    def permutation(self, n):
        return jax.random.permutation(self._next(), n)


kernel_name = 'gated_mix__softmax_full_mha__dense_activation_relu__prompt'

def setup_inputs():
    _rng = _Rng(jax.random.key(int.from_bytes(__import__("os").urandom(4), "little")))
    _w = (lambda a: (lambda t: t.astype(jnp.bfloat16) if jnp.issubdtype(t.dtype, jnp.floating) else t)(jnp.asarray(a)))
    def _A_setup():
        B, S, D = 1, 2048, 640
        return {
            "x": _w((lambda *s: _rng.normal(s) * 0.05)(B, S, D)),
            "wqkv": _w((lambda *s: _rng.normal(s) * 0.8)(D, 3 * D)),
            "wo": _w((lambda *s: _rng.normal(s) * 0.05)(D, D)),
        }
    _A_in = _A_setup()

    def _B_setup():
        B, S, D, Dff = 1, 2048, 640, 1536
        return {
            "x": _w((lambda *s: _rng.normal(s) * 0.05)(B, S, D)),
            "w1": _w((lambda *s: _rng.normal(s) * 0.05)(D, Dff)),
            "w2": _w((lambda *s: _rng.normal(s) * 0.05)(Dff, D)),
        }
    _B_in = _B_setup()

    return {
        "A_x": _A_in["x"],
        "A_wqkv": _A_in["wqkv"],
        "A_wo": _A_in["wo"],
        "B_x": _B_in["x"],
        "B_w1": _B_in["w1"],
        "B_w2": _B_in["w2"],
        "gate_w": _w((lambda *s: _rng.normal(s) * 0.05)(640) * 16.0),
    }

def reference(A_x, A_wqkv, A_wo, B_x, B_w1, B_w2, gate_w):
    def _A_ref(x, wqkv, wo):
        B, S, D = x.shape
        H = 32; Dh = D // H
        qkv = (lambda x, *d: x.transpose(*d))((x @ wqkv).reshape(B, S, 3, H, Dh), 2, 0, 3, 1, 4)
        q, k, v = qkv[0], qkv[1], qkv[2]
        scale = Dh ** -0.5
        scores = jnp.einsum("bhqd,bhkd->bhqk", q, k) * scale
        p = _softmax(scores, axis=-1)
        o = jnp.einsum("bhqk,bhkd->bhqd", p, v)
        return (lambda x, *d: x.transpose(*d))(o, 0, 2, 1, 3).reshape(B, S, D) @ wo

    def _B_ref(x, w1, w2):
        h = jnp.einsum("bsd,df->bsf", x, w1)
        zero = jnp.zeros_like(h)
        h = jnp.maximum(h, zero)
        return jnp.einsum("bsf,fd->bsd", h, w2)

    x = A_x
    g = _sigmoid((x * gate_w).sum(-1, keepdims=True))
    a = _A_ref(x, A_wqkv, A_wo)
    b = _B_ref(x, B_w1, B_w2)
    return g * a + (1 - g) * b
```

```python
import functools
import math

import jax
import jax.numpy as jnp
import jax.experimental.pallas as pl
import jax.experimental.pallas.tpu as pltpu

_H = 32
_HPT = 6
_LOG2E = math.log2(math.e)
_L_MIN = 2.0 ** -80

_NN = (((1,), (0,)), ((), ()))
_NT = (((1,), (1,)), ((), ()))


def _dot(a, b, dims=_NN):
    return jax.lax.dot_general(a, b, dims, preferred_element_type=jnp.float32)


def _iota(shape, dim):
    return jax.lax.broadcasted_iota(jnp.int32, shape, dim)


def _kernel(x_hbm, wqkv_hbm, wo_hbm, w1_hbm, w2_hbm, gw_ref, out_hbm,
            x_v, wqkv_v, wo_v, w1_v, w2_v, wt_s, k_s, qt_s, vt_s, m_s, kn_s, ot_s, out_v,
            in_sems, out_sems, *, S, D, RB, CK, LAG):
    f32, bf16 = jnp.float32, jnp.bfloat16
    Dh = D // _H
    GW = _HPT * Dh
    NG = -(-_H // _HPT)
    NB = S // RB
    qscale = Dh ** -0.5 * _LOG2E

    def x_copy(b):
        return pltpu.make_async_copy(x_hbm.at[pl.ds(b * RB, RB)], x_v.at[pl.ds(b * RB, RB)],
                                     in_sems.at[b])

    def w_copy(j):
        return pltpu.make_async_copy(wqkv_hbm.at[:, pl.ds(j * D, D)], wqkv_v.at[j],
                                     in_sems.at[NB + j])

    late = [pltpu.make_async_copy(src, dst, in_sems.at[NB + 3 + i])
            for i, (src, dst) in enumerate(((w1_hbm, w1_v), (w2_hbm, w2_v), (wo_hbm, wo_v)))]

    w_copy(0).start()
    w_copy(2).start()
    x_copy(0).start()
    w_copy(1).start()
    for b in range(1, NB):
        x_copy(b).start()
    for c in late:
        c.start()

    w_copy(0).wait()
    wt_s[0:D, :] = wqkv_v[0].T
    w_copy(2).wait()
    wt_s[D:2 * D, :] = wqkv_v[2].T
    qt_s[D:, :] = jnp.zeros((qt_s.shape[0] - D, S), f32)
    kn_s[...] = jnp.zeros(kn_s.shape, f32)
    w_copy(1).wait()

    def project(b, carry):
        x_copy(b).wait()
        r0 = pl.multiple_of(b * RB, RB)
        xb = x_v[pl.ds(r0, RB), :]
        qv = _dot(wt_s[...], xb, _NT)
        kb = _dot(xb, wqkv_v[1]).astype(bf16)

        q = (qv[0:D] * qscale).astype(bf16).astype(f32)
        qt_s[0:D, pl.ds(r0, RB)] = q
        ind = (_iota((_H, D), 1) // Dh == _iota((_H, D), 0)).astype(bf16)
        m_s[:, pl.ds(r0, RB)] = _dot(ind, (q * q).astype(bf16))

        v = qv[D:2 * D].astype(bf16).astype(f32)
        sub = _iota((8, RB), 0)
        for p in range(_H // 2):
            base = 2 * Dh * p
            mid = v[base + 16:base + 24]
            vt_s[2 * p, 0:16, pl.ds(r0, RB)] = v[base:base + 16]
            vt_s[2 * p, 16:24, pl.ds(r0, RB)] = jnp.where(sub < 4, mid, 1.0)
            vt_s[2 * p + 1, 0:8, pl.ds(r0, RB)] = jnp.where(sub < 4, 1.0, mid)
            vt_s[2 * p + 1, 8:24, pl.ds(r0, RB)] = v[base + 24:base + 40]

        kf = kb.astype(f32)
        lane = _iota((RB, 128), 1)
        for g in range(NG):
            w = min(GW, D - g * GW)
            t = kf[:, g * GW:g * GW + w]
            t = jnp.concatenate([t, jnp.ones((RB, 128 - w), f32)], axis=1)
            k_s[g, pl.ds(r0, RB), :] = t.astype(bf16)
        kn = _dot(ind, (kf * kf).astype(bf16), _NT)
        kn_s[...] = jnp.maximum(kn_s[...], kn)
        return carry

    jax.lax.fori_loop(0, NB, project, 0)

    kmax = jnp.max(kn_s[...], axis=1, keepdims=True)
    m_s[...] = jnp.sqrt(m_s[...] * kmax) * 1.02

    def q_tile(h, shift):
        g = h // _HPT
        lo = (h - g * _HPT) * Dh
        row = _iota((128, S), 0)
        qt = qt_s[pl.ds(pl.multiple_of(g * GW, 8), 128), :]
        rest = jnp.where(row == GW, -shift, 0.0) if shift is not None else 0.0
        return g, jnp.where((row >= lo) & (row < lo + Dh), qt, rest).astype(bf16)

    def denom(h, acc):
        return jnp.where(h % 2 == 0, acc[20:21], acc[0:1])

    def head(h, bad):
        g, qt = q_tile(h, m_s[pl.ds(h, 1), :])
        n = S // CK
        acc = None
        ps = {}
        for c in range(n + LAG):
            if c < n:
                s = _dot(k_s[g, c * CK:(c + 1) * CK, :], qt)
                ps[c] = jnp.exp2(s).astype(bf16)
            if c >= LAG:
                j = c - LAG
                o = _dot(vt_s[h, :, j * CK:(j + 1) * CK], ps.pop(j))
                acc = o if acc is None else acc + o
        ot_s[h] = acc
        l = denom(h, acc)
        return jnp.maximum(bad, jnp.where(l >= _L_MIN, 0.0, 1.0))

    bad = jax.lax.fori_loop(0, _H, head, jnp.zeros((1, S), f32))

    @pl.when(jnp.max(bad) > 0.0)
    def _():
        def exact_head(h, carry):
            g, qt = q_tile(h, None)

            def scores(c):
                return _dot(k_s[g, pl.ds(pl.multiple_of(c * 128, 128), 128), :], qt)

            def max_step(c, m):
                return jnp.maximum(m, jnp.max(scores(c), axis=0, keepdims=True))

            m = jax.lax.fori_loop(0, S // 128, max_step, jnp.full((1, S), -jnp.inf, f32))

            def pv_step(c, acc):
                p = jnp.exp2(scores(c) - m).astype(bf16)
                return acc + _dot(vt_s[h, :, pl.ds(pl.multiple_of(c * 128, 128), 128)], p)

            ot_s[h] = jax.lax.fori_loop(0, S // 128, pv_step, jnp.zeros((24, S), f32))
            return carry

        jax.lax.fori_loop(0, _H, exact_head, 0)

    for c in late:
        c.wait()

    def out_copy(b):
        return pltpu.make_async_copy(out_v.at[pl.ds(b * RB, RB)], out_hbm.at[pl.ds(b * RB, RB)],
                                     out_sems.at[b])

    def finish(b, carry):
        r0 = pl.multiple_of(b * RB, RB)
        xb = x_v[pl.ds(r0, RB), :]
        hid = jnp.maximum(_dot(xb, w1_v[...]), 0.0).astype(bf16)
        ffn = _dot(hid, w2_v[...])
        sub = _iota((8, RB), 0)
        parts = []
        for p in range(_H // 2):
            e = ot_s[2 * p, :, pl.ds(r0, RB)]
            o = ot_s[2 * p + 1, :, pl.ds(r0, RB)]
            e = e * (1.0 / e[20:21])
            o = o * (1.0 / o[0:1])
            parts += [e[0:16], jnp.where(sub < 4, e[16:24], o[0:8]), o[8:24]]
        ot = jnp.concatenate(parts, axis=0).astype(bf16)
        att = _dot(ot.T, wo_v[...])
        z = jnp.sum(xb.astype(f32) * gw_ref[...].astype(f32), axis=1, keepdims=True)
        gate = 1.0 / (1.0 + jnp.exp(-z))
        out_v[pl.ds(r0, RB), :] = (gate * att + (1.0 - gate) * ffn).astype(out_v.dtype)
        out_copy(b).start()
        return carry

    jax.lax.fori_loop(0, NB, finish, 0)
    for b in range(NB):
        out_copy(b).wait()


def make(RB=512, CK=128, LAG=1):
    @jax.jit
    def fn(A_x, A_wqkv, A_wo, B_x, B_w1, B_w2, gate_w):
        del B_x
        B, S, D = A_x.shape
        Dff = B_w1.shape[1]
        assert B == 1 and D == 20 * _H
        NB = S // RB
        NG = -(-_H // _HPT)
        f32, bf16 = jnp.float32, jnp.bfloat16
        hbm = pl.BlockSpec(memory_space=pl.ANY)
        out = pl.pallas_call(
            functools.partial(_kernel, S=S, D=D, RB=RB, CK=CK, LAG=LAG),
            out_shape=jax.ShapeDtypeStruct((S, D), A_x.dtype),
            in_specs=[hbm] * 5 + [pl.BlockSpec(memory_space=pltpu.VMEM)],
            out_specs=hbm,
            scratch_shapes=[
                pltpu.VMEM((S, D), bf16),
                pltpu.VMEM((3, D, D), bf16),
                pltpu.VMEM((D, D), bf16),
                pltpu.VMEM((D, Dff), bf16),
                pltpu.VMEM((Dff, D), bf16),
                pltpu.VMEM((2 * D, D), bf16),
                pltpu.VMEM((NG, S, 128), bf16),
                pltpu.VMEM(((NG - 1) * _HPT * 20 + 128, S), f32),
                pltpu.VMEM((_H, 24, S), f32),
                pltpu.VMEM((_H, S), f32),
                pltpu.VMEM((_H, RB), f32),
                pltpu.VMEM((_H, 24, S), f32),
                pltpu.VMEM((S, D), A_x.dtype),
                pltpu.SemaphoreType.DMA((NB + 6,)),
                pltpu.SemaphoreType.DMA((NB,)),
            ],
            compiler_params=pltpu.CompilerParams(vmem_limit_bytes=100 * 2 ** 20),
        )(A_x.reshape(S, D), A_wqkv, A_wo, B_w1, B_w2, gate_w.reshape(1, D))
        return out.reshape(B, S, D)
    return fn


pallas_gated_mix__softmax_full_mha__dense_activation_relu__prompt_kernel = make(**dict())
```

```python
import functools
import math

import jax
import jax.numpy as jnp
import jax.experimental.pallas as pl
import jax.experimental.pallas.tpu as pltpu

_H = 32
_HPT = 6
_LOG2E = math.log2(math.e)
_L_MIN = 2.0 ** -80

_NN = (((1,), (0,)), ((), ()))
_NT = (((1,), (1,)), ((), ()))


def _dot(a, b, dims=_NN):
    return jax.lax.dot_general(a, b, dims, preferred_element_type=jnp.float32)


def _dot_balanced(a, w_ref):
    n = a.shape[0] // 4
    last = [_dot(a[i * n:(i + 1) * n], w_ref[:, 512:]) for i in range(4)]
    return jnp.concatenate([_dot(a, w_ref[:, :512]), jnp.concatenate(last, axis=0)], axis=1)


def _iota(shape, dim):
    return jax.lax.broadcasted_iota(jnp.int32, shape, dim)


def _kernel(x_hbm, wqkv_hbm, wo_hbm, w1_hbm, w2_hbm, gw_ref, out_hbm,
            x_v, wqkv_v, wo_v, w1_v, w2_v, wt_s, k_s, qt_s, vt_s, m_s, km_s, kr_s, ot_s, out_v,
            in_sems, out_sems, *, S, D, RB, CK, LAG, UN, CB, PU, FB, FU):
    f32, bf16 = jnp.float32, jnp.bfloat16
    Dh = D // _H
    GW = _HPT * Dh
    NG = -(-_H // _HPT)
    NB = S // RB
    qscale = Dh ** -0.5 * _LOG2E

    rest = (S - 2 * RB) // NB
    head_rows = ((0, RB // 2), (RB // 2, RB), (3 * RB // 2, RB // 2))

    def x_copy(r0, n, i):
        return pltpu.make_async_copy(x_hbm.at[pl.ds(r0, n)], x_v.at[pl.ds(r0, n)], in_sems.at[i])

    def x_rest(b):
        return x_copy(pl.multiple_of(2 * RB + b * rest, rest), rest, b)

    x_head = [x_copy(r0, n, NB + 6 + i) for i, (r0, n) in enumerate(head_rows)]

    def w_copy(j):
        return pltpu.make_async_copy(wqkv_hbm.at[:, pl.ds(j * D, D)], wqkv_v.at[j],
                                     in_sems.at[NB + j])

    late = [pltpu.make_async_copy(src, dst, in_sems.at[NB + 3 + i])
            for i, (src, dst) in enumerate(((w1_hbm, w1_v), (w2_hbm, w2_v), (wo_hbm, wo_v)))]

    def project_k(r0, n):
        rows = pl.ds(r0, n)
        kr_s[rows, :] = _dot_balanced(x_v[rows, :], wqkv_v.at[1]).astype(bf16)

    for c in (w_copy(1), x_head[0], x_head[1], w_copy(0), x_head[2], w_copy(2),
              *[x_rest(b) for b in range(NB)], *late):
        c.start()
    w_copy(1).wait()
    x_head[0].wait()
    project_k(*head_rows[0])
    x_head[1].wait()
    project_k(*head_rows[1])
    w_copy(0).wait()
    x_head[2].wait()
    w_copy(2).wait()
    project_k(*head_rows[2])
    wt_s[0:D, :] = wqkv_v[0].T
    wt_s[D:2 * D, :] = wqkv_v[2].T

    def project(b, kn):
        x_rest(b).wait()
        project_k(pl.multiple_of(2 * RB + b * rest, rest), rest)
        cols = pl.ds(pl.multiple_of(b * RB, RB), RB)
        xb = x_v[cols, :]
        ind = (_iota((_H, D), 1) // Dh == _iota((_H, D), 0)).astype(bf16)
        q = (_dot(wt_s[0:D, :], xb, _NT) * qscale).astype(bf16).astype(f32)
        qt_s[0:D, cols] = q
        kf = kr_s[cols, :].astype(f32)
        for g in range(NG):
            w = min(GW, D - g * GW)
            t = jnp.concatenate([kf[:, g * GW:g * GW + w], jnp.ones((RB, 128 - w), f32)], axis=1)
            k_s[g, cols, :] = t.astype(bf16)
        kn = jnp.maximum(kn, _dot(ind, (kf * kf).astype(bf16), _NT))
        v0 = _dot(wt_s[D:D + D // 2, :], xb, _NT)
        m_s[:, cols] = jnp.sqrt(_dot(ind, (q * q).astype(bf16)))
        v1 = _dot(wt_s[D + D // 2:, :], xb, _NT)
        v = jnp.concatenate([v0, v1], axis=0).astype(bf16).astype(f32)
        sub = _iota((8, RB), 0)
        for p in range(_H // 2):
            base = 2 * Dh * p
            mid = v[base + 16:base + 24]
            vt_s[2 * p, 0:16, cols] = v[base:base + 16]
            vt_s[2 * p, 16:24, cols] = jnp.where(sub < 4, mid, 1.0)
            vt_s[2 * p + 1, 0:8, cols] = jnp.where(sub < 4, 1.0, mid)
            vt_s[2 * p + 1, 8:24, cols] = v[base + 24:base + 40]
        return kn

    kn = jax.lax.fori_loop(0, NB, project, jnp.zeros((_H, RB), f32))
    km_s[...] = jnp.broadcast_to(jnp.sqrt(jnp.max(kn, axis=1, keepdims=True)) * -1.02, km_s.shape)

    def q_tile(h, shifted, cols):
        g = h // _HPT
        lo = (h - g * _HPT) * Dh
        qt = qt_s[pl.ds(pl.multiple_of(g * GW, 8), 128), cols]
        row = _iota(qt.shape, 0)
        rest = jnp.where(row == GW, m_s[pl.ds(h, 1), cols] * km_s[pl.ds(h, 1), :], 0.0) if shifted else 0.0
        return g, jnp.where((row >= lo) & (row < lo + Dh), qt, rest).astype(bf16)

    def emit(pair, odd, cols, acc):
        base = pl.multiple_of(pair * (2 * Dh), 8)
        l = acc[0:1] if odd else acc[20:21]
        o = acc * (1.0 / l)
        if odd:
            sub = _iota((8, acc.shape[1]), 0)
            shared = ot_s[pl.ds(base + 16, 8), cols]
            ot_s[pl.ds(base + 16, 8), cols] = jnp.where(sub < 4, shared, o[0:8])
            ot_s[pl.ds(base + 24, 16), cols] = o[8:24]
        else:
            ot_s[pl.ds(base, 24), cols] = o
        return l

    def heads(i, bad):
        n = S // 128
        tiles = [(u, j, c) for u in range(UN) for j in range(S // CB) for c in range(n)]
        ps, acc, done = {}, None, 0
        widths = {sum(CK[:e]): w for e, w in enumerate(CK)}
        t = 0
        while done < len(tiles):
            if t < len(tiles):
                u, j, c = tiles[t]
                if c == 0:
                    g, qt = q_tile(i * UN + u, True, slice(j * CB, (j + 1) * CB))
                w = widths[c]
                s = _dot(k_s[g, c * 128:(c + w) * 128, :], qt)
                for r in range(w):
                    ps[t + r] = jnp.exp2(s[r * 128:(r + 1) * 128]).astype(bf16)
                t += w
                upto = t - LAG
            else:
                upto = len(tiles)
            while done < upto:
                u, j, c = tiles[done]
                h = i * UN + u
                o = _dot(vt_s[h, :, c * 128:(c + 1) * 128], ps.pop(done))
                acc = o if c == 0 else acc + o
                if c == n - 1:
                    l = emit(i * (UN // 2) + u // 2, u % 2, slice(j * CB, (j + 1) * CB), acc)
                    bad = jnp.maximum(bad, jnp.where(l >= _L_MIN, 0.0, 1.0))
                done += 1
        return bad

    bad = jax.lax.fori_loop(0, _H // UN, heads, jnp.zeros((1, CB), f32))

    @pl.when(jnp.max(bad) > 0.0)
    def _():
        def exact(i, carry):
            h = i // (S // CB)
            cols = pl.ds(pl.multiple_of(i % (S // CB) * CB, CB), CB)
            g, qt = q_tile(h, False, cols)

            def scores(c):
                return _dot(k_s[g, pl.ds(pl.multiple_of(c * 128, 128), 128), :], qt)

            def max_step(c, m):
                return jnp.maximum(m, jnp.max(scores(c), axis=0, keepdims=True))

            m = jax.lax.fori_loop(0, S // 128, max_step, jnp.full((1, CB), -jnp.inf, f32))

            def pv_step(c, acc):
                p = jnp.exp2(scores(c) - m).astype(bf16)
                return acc + _dot(vt_s[h, :, pl.ds(pl.multiple_of(c * 128, 128), 128)], p)

            acc = jax.lax.fori_loop(0, S // 128, pv_step, jnp.zeros((24, CB), f32))
            for odd in (0, 1):
                @pl.when(h % 2 == odd)
                def _():
                    emit(h // 2, odd, cols, acc)
            return carry

        jax.lax.fori_loop(0, _H * (S // CB), exact, 0)

    for c in late:
        c.wait()

    def out_copy(b):
        rows = pl.ds(pl.multiple_of(b * FB, FB), FB)
        return pltpu.make_async_copy(out_v.at[rows], out_hbm.at[rows], out_sems.at[b])

    def finish_block(b):
        rows = pl.ds(pl.multiple_of(b * FB, FB), FB)
        xb = x_v[rows, :]
        hid = jnp.maximum(_dot(xb, w1_v[...]), 0.0).astype(bf16)
        ot = ot_s[:, rows].astype(bf16)
        att = _dot(ot.T, wo_v[...])
        ffn = _dot(hid, w2_v[...])
        z = jnp.sum(xb.astype(f32) * gw_ref[...].astype(f32).reshape(1, D), axis=1, keepdims=True)
        gate = 1.0 / (1.0 + jnp.exp(-z))
        out_v[rows, :] = (gate * att + (1.0 - gate) * ffn).astype(out_v.dtype)
        out_copy(b).start()

    def finish(i, carry):
        for u in range(FU):
            finish_block(i * FU + u)
        return carry

    jax.lax.fori_loop(0, S // FB // FU, finish, 0)
    for b in range(S // FB):
        out_copy(b).wait()


def make(RB=512, CK=(4, 4, 4, 4), LAG=1, UN=4, CB=512, PU=1, FB=512, FU=1, flags={'XLA_TPU_EVENLY_DISTRIBUTE_CRITICAL_NODES': True}):
    @jax.jit
    def fn(A_x, A_wqkv, A_wo, B_x, B_w1, B_w2, gate_w):
        del B_x
        B, S, D = A_x.shape
        Dff = B_w1.shape[1]
        assert B == 1 and D == 20 * _H
        NB = S // RB
        NG = -(-_H // _HPT)
        f32, bf16 = jnp.float32, jnp.bfloat16
        hbm = pl.BlockSpec(memory_space=pl.ANY)
        out = pl.pallas_call(
            functools.partial(_kernel, S=S, D=D, RB=RB, CK=CK, LAG=LAG, UN=UN, CB=CB, PU=PU, FB=FB, FU=FU),
            out_shape=jax.ShapeDtypeStruct((S, D), A_x.dtype),
            in_specs=[hbm] * 5 + [pl.BlockSpec(memory_space=pltpu.VMEM)],
            out_specs=hbm,
            scratch_shapes=[
                pltpu.VMEM((S, D), bf16),
                pltpu.VMEM((3, D, D), bf16),
                pltpu.VMEM((D, D), bf16),
                pltpu.VMEM((D, Dff), bf16),
                pltpu.VMEM((Dff, D), bf16),
                pltpu.VMEM((2 * D, D), bf16),
                pltpu.VMEM((NG, S, 128), bf16),
                pltpu.VMEM(((NG - 1) * _HPT * 20 + 128, S), f32),
                pltpu.VMEM((_H, 24, S), f32),
                pltpu.VMEM((_H, S), f32),
                pltpu.VMEM((_H, CB), f32),
                pltpu.VMEM((S, D), bf16),
                pltpu.VMEM((D, S), f32),
                pltpu.VMEM((S, D), A_x.dtype),
                pltpu.SemaphoreType.DMA((NB + 9,)),
                pltpu.SemaphoreType.DMA((S // FB,)),
            ],
            compiler_params=pltpu.CompilerParams(vmem_limit_bytes=100 * 2 ** 20, flags=flags),
        )(A_x.reshape(S, D), A_wqkv, A_wo, B_w1, B_w2, gate_w)
        return out.reshape(B, S, D)
    return fn


pallas_gated_mix__softmax_full_mha__dense_activation_relu__prompt_kernel = make(**dict(CK=(4, 3, 3, 3, 3), LAG=1, flags=None))
```

```python
import functools
import math

import jax
import jax.numpy as jnp
import jax.experimental.pallas as pl
import jax.experimental.pallas.tpu as pltpu

_H = 32
_DH = 20
_HPT = 6
_GW = _HPT * _DH
_NG = -(-_H // _HPT)

_RB = 512
_CB = 512
_HEADS = 4
_QK_TILES = (4, 3, 3, 3, 3)
_LAG = 1
_FB = 128
_FU = 8

_NN = (((1,), (0,)), ((), ()))
_NT = (((1,), (1,)), ((), ()))


def _dot(a, b, dims=_NN):
    return jax.lax.dot_general(a, b, dims, preferred_element_type=jnp.float32)


def _dot_balanced(a, w_ref):
    n = a.shape[0] // 4
    last = [_dot(a[i * n:(i + 1) * n], w_ref[:, 512:]) for i in range(4)]
    return jnp.concatenate([_dot(a, w_ref[:, :512]), jnp.concatenate(last, axis=0)], axis=1)


def _iota(shape, dim):
    return jax.lax.broadcasted_iota(jnp.int32, shape, dim)


def _kernel(x_hbm, wqkv_hbm, wo_hbm, w1_hbm, w2_hbm, gw_ref, out_hbm,
            x_v, wqkv_v, wo_v, w1_v, w2_v, wt_s, kr_s, k_s, qt_s, vt_s, qn_s, kn_s, ot_s,
            gate_s, ffn_s, out_v, in_sems, out_sems):
    f32, bf16 = jnp.float32, jnp.bfloat16
    S, D = x_v.shape
    NB = S // _RB
    qscale = _DH ** -0.5 * math.log2(math.e)

    first_rows = ((0, _RB // 2), (_RB // 2, _RB), (3 * _RB // 2, _RB // 2))
    rest = (S - 2 * _RB) // NB

    def x_copy(r0, n, i):
        return pltpu.make_async_copy(x_hbm.at[pl.ds(r0, n)], x_v.at[pl.ds(r0, n)], in_sems.at[i])

    def rest_start(b):
        return pl.multiple_of(2 * _RB + b * rest, rest)

    x_first = [x_copy(r0, n, NB + i) for i, (r0, n) in enumerate(first_rows)]
    wq_copy, wk_copy, wv_copy = [
        pltpu.make_async_copy(wqkv_hbm.at[:, pl.ds(j * D, D)], wqkv_v.at[j], in_sems.at[NB + 3 + j])
        for j in range(3)]
    w1_copy, w2_copy, wo_copy = [
        pltpu.make_async_copy(src, dst, in_sems.at[NB + 6 + i])
        for i, (src, dst) in enumerate(((w1_hbm, w1_v), (w2_hbm, w2_v), (wo_hbm, wo_v)))]

    for c in (wk_copy, x_first[0], x_first[1], wq_copy, x_first[2], wv_copy,
              *[x_copy(rest_start(b), rest, b) for b in range(NB)], w1_copy, w2_copy, wo_copy):
        c.start()

    def project_k(r0, n):
        rows = pl.ds(r0, n)
        kr_s[rows, :] = _dot_balanced(x_v[rows, :], wqkv_v.at[1]).astype(bf16)

    qt_s[D:, :] = jnp.zeros((qt_s.shape[0] - D, S), f32)
    wk_copy.wait()
    x_first[0].wait()
    project_k(*first_rows[0])
    x_first[1].wait()
    project_k(*first_rows[1])
    wq_copy.wait()
    x_first[2].wait()
    wv_copy.wait()
    project_k(*first_rows[2])
    wt_s[0:D, :] = wqkv_v[0].T
    wt_s[D:2 * D, :] = wqkv_v[2].T

    def project(b, kn):
        x_copy(rest_start(b), rest, b).wait()
        project_k(rest_start(b), rest)
        cols = pl.ds(pl.multiple_of(b * _RB, _RB), _RB)
        xb = x_v[cols, :]
        q = (_dot(wt_s[0:D, :], xb, _NT) * qscale).astype(bf16).astype(f32)
        qt_s[0:D, cols] = q

        kb = kr_s[cols, :]
        for g in range(_NG):
            w = min(_GW, D - g * _GW)
            k_s[g, cols, :] = jnp.concatenate(
                [kb[:, g * _GW:g * _GW + w], jnp.ones((_RB, 128 - w), bf16)], axis=1)
        kf = kb.astype(f32)
        v0 = _dot(wt_s[D:D + D // 2, :], xb, _NT)
        head_of = (_iota((_H, D), 1) // _DH == _iota((_H, D), 0)).astype(bf16)
        kn = jnp.maximum(kn, _dot(head_of, (kf * kf).astype(bf16), _NT))

        low = _iota((8, _RB), 0) < 4
        for p in range(_H // 2):
            sq = q[2 * _DH * p:2 * _DH * (p + 1)] ** 2
            even = sq[0:8] + sq[8:16] + jnp.where(low, sq[16:24], 0.0)
            odd = jnp.where(low, 0.0, sq[16:24]) + sq[24:32] + sq[32:40]
            qn_s[2 * p:2 * p + 1, cols] = jnp.sum(even, axis=0, keepdims=True)
            qn_s[2 * p + 1:2 * p + 2, cols] = jnp.sum(odd, axis=0, keepdims=True)
        qn_s[:, cols] = jnp.sqrt(qn_s[:, cols])

        v1 = _dot(wt_s[D + D // 2:, :], xb, _NT)
        v = jnp.concatenate([v0, v1], axis=0).astype(bf16).astype(f32)
        for p in range(_H // 2):
            base = 2 * _DH * p
            mid = v[base + 16:base + 24]
            vt_s[2 * p, 0:16, cols] = v[base:base + 16]
            vt_s[2 * p, 16:24, cols] = jnp.where(low, mid, 1.0)
            vt_s[2 * p + 1, 0:8, cols] = jnp.where(low, 1.0, mid)
            vt_s[2 * p + 1, 8:24, cols] = v[base + 24:base + 40]
        return kn

    kn = jax.lax.fori_loop(0, NB, project, jnp.zeros((_H, _RB), f32))
    kn_s[...] = jnp.broadcast_to(jnp.sqrt(jnp.max(kn, axis=1, keepdims=True)) * -1.02, kn_s.shape)

    def q_tile(h, cols, shift):
        g = h // _HPT
        lo = (h - g * _HPT) * _DH
        qt = qt_s[pl.ds(pl.multiple_of(g * _GW, 8), 128), cols]
        row = _iota(qt.shape, 0)
        other = jnp.where(row == _GW, shift, 0.0)
        return g, jnp.where((row >= lo) & (row < lo + _DH), qt, other).astype(bf16)

    def denominator(odd, acc):
        return acc[0:1] if odd else acc[20:21]

    def emit(pair, odd, cols, acc):
        base = pl.multiple_of(pair * (2 * _DH), 8)
        o = acc * (1.0 / denominator(odd, acc))
        if odd:
            low = _iota((8, acc.shape[1]), 0) < 4
            shared = ot_s[pl.ds(base + 16, 8), cols]
            ot_s[pl.ds(base + 16, 8), cols] = jnp.where(low, shared, o[0:8])
            ot_s[pl.ds(base + 24, 16), cols] = o[8:24]
        else:
            ot_s[pl.ds(base, 24), cols] = o

    def unsafe(odd, acc):
        tiny = jnp.where(jnp.abs(acc) >= 2.0 ** -80, 0.0, 1.0)
        tiny = jnp.maximum(jnp.maximum(tiny[0:8], tiny[8:16]), tiny[16:24])
        return tiny * jnp.where(denominator(odd, acc) >= 2.0 ** -12, 0.0, 1.0)

    w1_copy.wait()
    w2_copy.wait()

    def attend(i, bad):
        n = S // 128
        fr = S * _HEADS // _H
        rows = pl.ds(pl.multiple_of(i * fr, fr), fr)
        tiles = [(u, j, c) for u in range(_HEADS) for j in range(S // _CB) for c in range(n)]
        widths = {sum(_QK_TILES[:e]): w for e, w in enumerate(_QK_TILES)}
        probs, acc, scored, summed = {}, None, 0, 0
        while summed < len(tiles):
            if scored < len(tiles):
                u, j, c = tiles[scored]
                if c == 0:
                    h, cols = i * _HEADS + u, slice(j * _CB, (j + 1) * _CB)
                    g, qt = q_tile(h, cols, qn_s[pl.ds(h, 1), cols] * kn_s[pl.ds(h, 1), :])
                s = _dot(k_s[g, c * 128:(c + widths[c]) * 128, :], qt)
                for r in range(widths[c]):
                    probs[scored + r] = jnp.exp2(s[r * 128:(r + 1) * 128]).astype(bf16)
                scored += widths[c]
                ready = scored - _LAG
            else:
                hid = jnp.maximum(_dot(x_v[rows, :], w1_v[...]), 0.0).astype(bf16)
                ready = len(tiles)
            while summed < ready:
                u, j, c = tiles[summed]
                o = _dot(vt_s[i * _HEADS + u, :, c * 128:(c + 1) * 128], probs.pop(summed))
                acc = o if c == 0 else acc + o
                if c == n - 1:
                    emit(i * (_HEADS // 2) + u // 2, u % 2, slice(j * _CB, (j + 1) * _CB), acc)
                    bad = jnp.maximum(bad, unsafe(u % 2, acc))
                summed += 1
        z = jnp.sum(x_v[rows, :].astype(f32) * gw_ref[...].astype(f32).reshape(1, D),
                    axis=1, keepdims=True)
        gate = 1.0 / (1.0 + jnp.exp(-z))
        gate_s[rows, :] = jnp.broadcast_to(gate, (fr, 128))
        ffn_s[rows, :] = (1.0 - gate) * _dot(hid, w2_v[...])
        return bad

    bad = jax.lax.fori_loop(0, _H // _HEADS, attend, jnp.zeros((8, _CB), f32))

    @pl.when(jnp.max(bad) > 0.0)
    def _():
        def attend_true_max(i, carry):
            h = i // (S // _CB)
            cols = pl.ds(pl.multiple_of(i % (S // _CB) * _CB, _CB), _CB)
            g, qt = q_tile(h, cols, 0.0)

            def keys(c):
                return pl.ds(pl.multiple_of(c * 128, 128), 128)

            def max_step(c, m):
                return jnp.maximum(m, jnp.max(_dot(k_s[g, keys(c), :], qt), axis=0, keepdims=True))

            m = jax.lax.fori_loop(0, S // 128, max_step, jnp.full((1, _CB), -jnp.inf, f32))

            def pv_step(c, acc):
                p = jnp.exp2(_dot(k_s[g, keys(c), :], qt) - m).astype(bf16)
                return acc + _dot(vt_s[h, :, keys(c)], p)

            acc = jax.lax.fori_loop(0, S // 128, pv_step, jnp.zeros((24, _CB), f32))
            for odd in (0, 1):
                pl.when(h % 2 == odd)(functools.partial(emit, h // 2, odd, cols, acc))
            return carry

        jax.lax.fori_loop(0, _H * (S // _CB), attend_true_max, 0)

    wo_copy.wait()

    def out_rows(b):
        return pl.ds(pl.multiple_of(b * _FB, _FB), _FB)

    def out_copy(b):
        return pltpu.make_async_copy(out_v.at[out_rows(b)], out_hbm.at[out_rows(b)], out_sems.at[b])

    def finish(i, carry):
        for u in range(_FU):
            b = i * _FU + u
            rows = out_rows(b)
            att = _dot(ot_s[:, rows].astype(bf16).T, wo_v[...])
            gate = jnp.concatenate([gate_s[rows, :]] * (D // 128), axis=1)
            out_v[rows, :] = (gate * att + ffn_s[rows, :]).astype(out_v.dtype)
            out_copy(b).start()
        return carry

    jax.lax.fori_loop(0, S // _FB // _FU, finish, 0)
    for b in range(S // _FB):
        out_copy(b).wait()


@jax.jit
def pallas_gated_mix__softmax_full_mha__dense_activation_relu__prompt_kernel(
    A_x: jax.Array,
    A_wqkv: jax.Array,
    A_wo: jax.Array,
    B_x: jax.Array,
    B_w1: jax.Array,
    B_w2: jax.Array,
    gate_w: jax.Array,
):
    del B_x
    B, S, D = A_x.shape
    Dff = B_w1.shape[1]
    assert (B, S, D) == (1, 128 * sum(_QK_TILES), _H * _DH)
    f32, bf16 = jnp.float32, jnp.bfloat16
    hbm = pl.BlockSpec(memory_space=pl.ANY)
    out = pl.pallas_call(
        _kernel,
        out_shape=jax.ShapeDtypeStruct((S, D), A_x.dtype),
        in_specs=[hbm] * 5 + [pl.BlockSpec(memory_space=pltpu.VMEM)],
        out_specs=hbm,
        scratch_shapes=[
            pltpu.VMEM((S, D), bf16),
            pltpu.VMEM((3, D, D), bf16),
            pltpu.VMEM((D, D), bf16),
            pltpu.VMEM((D, Dff), bf16),
            pltpu.VMEM((Dff, D), bf16),
            pltpu.VMEM((2 * D, D), bf16),
            pltpu.VMEM((S, D), bf16),
            pltpu.VMEM((_NG, S, 128), bf16),
            pltpu.VMEM(((_NG - 1) * _GW + 128, S), f32),
            pltpu.VMEM((_H, 24, S), f32),
            pltpu.VMEM((_H, S), f32),
            pltpu.VMEM((_H, _CB), f32),
            pltpu.VMEM((D, S), f32),
            pltpu.VMEM((S, 128), f32),
            pltpu.VMEM((S, D), f32),
            pltpu.VMEM((S, D), A_x.dtype),
            pltpu.SemaphoreType.DMA((S // _RB + 9,)),
            pltpu.SemaphoreType.DMA((S // _FB,)),
        ],
        compiler_params=pltpu.CompilerParams(vmem_limit_bytes=100 * 2 ** 20),
    )(A_x.reshape(S, D), A_wqkv, A_wo, B_w1, B_w2, gate_w)
    return out.reshape(B, S, D)
```
